```python
import os as _os
_os.environ.setdefault('JAX_PLATFORMS', 'cpu')
import jax
import jax.numpy as jnp

def _softmax(x, axis=-1):
    return jax.nn.softmax(x, axis=axis)

def _gelu(x):
    return jax.nn.gelu(x, approximate=True)

def _silu(x):
    return jax.nn.silu(x)

def _sigmoid(x):
    return jax.nn.sigmoid(x)

def _layernorm(x, axis=-1, eps=1e-05):
    m = jnp.mean(x, axis=axis, keepdims=True)
    v = jnp.var(x, axis=axis, keepdims=True)
    return (x - m) / jnp.sqrt(v + eps)

def _scatter_add(tgt, idx, src, axis=0):
    return tgt.at[idx].add(src)

def _segment_sum(src, seg, n):
    return jax.ops.segment_sum(src, seg, n)

class _Rng:

    def __init__(self, key):
        self._k = key

    def _next(self):
        self._k, sub = jax.random.split(self._k)
        return sub

    def normal(self, shape):
        return jax.random.normal(self._next(), shape, dtype=jnp.bfloat16)

    def randint(self, lo, hi, shape):
        return jax.random.randint(self._next(), shape, lo, hi, dtype=jnp.int32)

    def uniform(self, shape, lo=0.0, hi=1.0):
        return jax.random.uniform(self._next(), shape, jnp.bfloat16, lo, hi)

    def permutation(self, n):
        return jax.random.permutation(self._next(), n)
kernel_name = 'adaLN_cond__mha_block_cached__geglu_ffn__prompt'

def setup_inputs():
    _rng = _Rng(jax.random.key(int.from_bytes(__import__("os").urandom(4), "little")))
    _w = lambda a: (lambda t: t.astype(jnp.bfloat16) if jnp.issubdtype(t.dtype, jnp.floating) else t)(jnp.asarray(a))

    def _A_setup():
        B, Sq, D = (1, 2048, 512)
        H, Sk, Dh = (32, 2048, 128)
        return {'x': _w((lambda *s: _rng.normal(s) * 0.05)(B, Sq, D)), 'k_cache': _w((lambda *s: _rng.normal(s) * 3.2)(B, H, Sk, Dh)), 'v_cache': _w((lambda *s: _rng.normal(s) * 0.4)(B, H, Sk, Dh)), 'wq': _w((lambda *s: _rng.normal(s) * 1.6)(D, H * Dh) * D ** (-0.5)), 'wo': _w((lambda *s: _rng.normal(s) * 0.4)(H * Dh, D) * (H * Dh) ** (-0.5))}
    _A_in = _A_setup()

    def _B_setup():
        B, S, D, F = (1, 2048, 512, 1792)
        return {'x': _w((lambda *s: _rng.normal(s) * 0.05)(B, S, D)), 'w_gate': _w((lambda *s: _rng.normal(s) * 0.05)(D, F)), 'w_up': _w((lambda *s: _rng.normal(s) * 0.05)(D, F)), 'w_down': _w((lambda *s: _rng.normal(s) * 0.05)(F, D))}
    _B_in = _B_setup()
    return {'A_x': _A_in['x'], 'A_k_cache': _A_in['k_cache'], 'A_v_cache': _A_in['v_cache'], 'A_wq': _A_in['wq'], 'A_wo': _A_in['wo'], 'B_x': _B_in['x'], 'B_w_gate': _B_in['w_gate'], 'B_w_up': _B_in['w_up'], 'B_w_down': _B_in['w_down'], 'c': _w((lambda *s: _rng.normal(s) * 0.05)(1, 512) * 8.0), 'w_mod': _w((lambda *s: _rng.normal(s) * 0.05)(512, 6 * 512) * 512 ** (-0.5) * 8.0)}

def reference(A_x, A_k_cache, A_v_cache, A_wq, A_wo, B_x, B_w_gate, B_w_up, B_w_down, c, w_mod):

    def _A_ref(x, k_cache, v_cache, wq, wo):
        B, Sq, D = x.shape
        H, Dh = (32, 128)
        q = (lambda x, *d: x.transpose(*d))((x @ wq).reshape(B, Sq, H, Dh), 0, 2, 1, 3)
        scores = jnp.einsum('bhqd,bhkd->bhqk', q, k_cache) * Dh ** (-0.5)
        p = _softmax(scores, axis=-1)
        o = jnp.einsum('bhqk,bhkd->bhqd', p, v_cache)
        return (lambda x, *d: x.transpose(*d))(o, 0, 2, 1, 3).reshape(B, Sq, H * Dh) @ wo

    def _B_ref(x, w_gate, w_up, w_down):
        return _gelu(x @ w_gate) * (x @ w_up) @ w_down
    x = A_x
    mod = (_silu(c) @ w_mod).reshape(c.shape[0], 6, 1, -1)
    sa, ca, ga, sb, cb, gb = (mod[:, 0].copy(), mod[:, 1].copy(), mod[:, 2].copy(), mod[:, 3].copy(), mod[:, 4].copy(), mod[:, 5].copy())
    h = _layernorm(x, axis=-1) * (1 + ca) + sa
    x = x + ga * _A_ref(h, A_k_cache, A_v_cache, A_wq, A_wo)
    h = _layernorm(x, axis=-1) * (1 + cb) + sb
    x = x + gb * _B_ref(h, B_w_gate, B_w_up, B_w_down)
    return x
```

```python
import jax
import jax.numpy as jnp
import numpy as np
from jax import lax
import jax.experimental.pallas as pl
import jax.experimental.pallas.tpu as pltpu

_CFG = {'MERGE': '0', 'R': '512', 'RHO': '2', 'XWP': '0,1', 'QPJF': '0', 'FXJ': '1', 'DORD': '8', 'LSUML': '1', 'WAL': '2048', 'QPJL': '0', 'U32': '15', 'WAF': '2048', 'LSUMF': '1', 'WAE': '2048', 'LSUME': '1'}


class _E:
    @staticmethod
    def get(k, d=None):
        return _CFG.get(k, d)


def _env(n, d):
    return int(_E.get(n, d))

H, DH, S, D, F = 32, 128, 2048, 512, 1792
R = _env("R", 256)
W = _env("W", 512)
QPJ = _env("QPJ", 1)
FINJ = _env("FINJ", 1)
OPJ = _env("OPJ", 2)
RF = _env("RF", 256)
FW = _env("FW", 256)
LP = _env("LP", 1)
UH = _env("UH", 2)
ORD = _env("ORD", 0)
SCOPES = _env("SCOPES", 0)
LNP = _env("LNP", 2)
LN0 = _env("LN0", 2)
L1J = _env("L1J", 0)
L2J = _env("L2J", 0)
NSLOT = 4
SK = _env("SK", 0)
MERGE = _env("MERGE", 1)
PJ = _env("PJ", 1)
RHO = _env("RHO", 6)
MASK = NSLOT - 1
XR = 256
XC = S // XR
EPS = 1e-5
LOG2E = 1.4426950408889634
N = S // R
G = S // W
NF = S // RF
NG = F // FW
def _cfg(sfx):
    return (_env("QPJ" + sfx, QPJ), _env("FINJ" + sfx, FINJ), _env("OPJ" + sfx, OPJ), _env("ORD" + sfx, ORD),
            _env("MJ" + sfx, 0), _env("LSUM" + sfx, 0), _env("WA" + sfx, W),
            [int(v) for v in _E.get("AJ" + sfx).split(',')] if _E.get("AJ" + sfx) else None)
CFG_F, CFG_L, CFG_E = _cfg("F"), _cfg("L"), _cfg("E")
ONLY = _E.get("ONLY", "")
U32 = _env("U32", 0)
f32 = jnp.float32
bf16 = jnp.bfloat16


def _ld_packed(ref, slot, start, size):
    w = ref.bitcast(jnp.uint32)[slot, pl.ds(start // 2, size // 2), :]
    return pltpu.bitcast(w, bf16)


def _lane_tiles(x):
    return [x[:, i * 128:(i + 1) * 128] for i in range(x.shape[1] // 128)]


def _ln(x):
    m = jnp.mean(x, axis=-1, keepdims=True)
    xc = x - m
    v = jnp.mean(xc * xc, axis=-1, keepdims=True)
    return xc * lax.rsqrt(v + EPS)


def _recip(l):
    r = pl.reciprocal(l, approx=True)
    r = r * (2.0 - l * r)
    return r * (2.0 - l * r) if _env("RCP", 1) == 2 else r


class _Scope:
    def __init__(self):
        self.cur = None

    def __call__(self, name):
        if not SCOPES:
            return
        if self.cur is not None:
            self.cur.__exit__(None, None, None)
            self.cur = None
        if name:
            self.cur = jax.named_scope(name)
            self.cur.__enter__()


def _kernel(x_hbm, k_hbm, v_hbm, wq_hbm, wo_hbm, wg_hbm, wu_hbm, wd_hbm, c_hbm, wm_hbm, o_hbm,
            x_v, k_v, v_v, wq_v, wo_v, wg_v, wu_v, wd_v, c_v, wm_v, out_v,
            mod_v, sc_v, h_v, acc_v, s0_v, s1_v, m_c, q_c, o_c, l_c, h2_v, p0_v, p1_v,
            sem_head, sem_misc, sem_x, sem_out):
    scope = _Scope()
    fscope = scope if SCOPES == 2 else (lambda n: None)
    scale = (DH ** -0.5) * LOG2E
    s_refs = [s0_v, s1_v]
    p_refs = [p0_v, p1_v]

    def head_copies(h, slot):
        col = pl.multiple_of(h * DH, DH)
        return [
            pltpu.make_async_copy(wq_hbm.at[:, pl.ds(col, DH)], wq_v.at[slot], sem_head.at[0, slot]),
            pltpu.make_async_copy(k_hbm.at[h], k_v.at[slot], sem_head.at[1, slot]),
            pltpu.make_async_copy(v_hbm.at[h], v_v.at[slot], sem_head.at[2, slot]),
            pltpu.make_async_copy(wo_hbm.at[pl.ds(col, DH), :], wo_v.at[slot], sem_head.at[3, slot]),
        ]

    cp_c = pltpu.make_async_copy(c_hbm, c_v, sem_misc.at[0])
    cp_wm0 = pltpu.make_async_copy(wm_hbm.at[:, pl.ds(0, 2 * D)], wm_v.at[:, pl.ds(0, 2 * D)], sem_misc.at[1])
    cp_wm1 = pltpu.make_async_copy(wm_hbm.at[:, pl.ds(2 * D, 4 * D)], wm_v.at[:, pl.ds(2 * D, 4 * D)], sem_misc.at[2])
    cp_wg = pltpu.make_async_copy(wg_hbm, wg_v, sem_misc.at[3])
    cp_wu = pltpu.make_async_copy(wu_hbm, wu_v, sem_misc.at[4])
    cp_wd = pltpu.make_async_copy(wd_hbm, wd_v, sem_misc.at[5])
    cp_x = [pltpu.make_async_copy(x_hbm.at[pl.ds(i * XR, XR), :], x_v.at[pl.ds(i * XR, XR), :], sem_x.at[i])
            for i in range(XC)]
    x_waited = set()

    def x_wait(upto):
        for i in range(min(upto, XC - 1) + 1):
            if i not in x_waited:
                x_waited.add(i)
                cp_x[i].wait()

    def ln1(i):
        sa = mod_v[0:1, 0:D]
        ca1 = 1.0 + mod_v[0:1, D:2 * D]
        rows = pl.ds(i * R, R)
        hn = (_ln(x_v[rows, :].astype(f32)) * ca1 + sa).astype(bf16)
        if U32 & 8:
            for ct in range(D // 128):
                h_v.bitcast(jnp.uint32)[ct, pl.ds(i * R // 2, R // 2), :] = pltpu.bitcast(hn[:, ct * 128:(ct + 1) * 128], jnp.uint32)
        else:
            h_v[rows, :] = hn

    def qproj(slot, c):
        ww = _ld_packed(wq_v, slot, 0, D) if U32 & 4 else wq_v[slot]
        if U32 & 8:
            hh = jnp.concatenate([_ld_packed(h_v, ct, c * R, R) for ct in range(D // 128)], axis=1)
        else:
            hh = h_v[pl.ds(c * R, R), :]
        t = jnp.dot(hh, ww, preferred_element_type=f32)
        return (t * scale).astype(bf16)

    def score(q, slot, j, w, sref, z):
        kk = _ld_packed(k_v, slot, j * w, w) if U32 & 1 else k_v[slot, pl.ds(j * w, w), :]
        t = lax.dot_general(q, kk, (((1,), (1,)), ((), ())),
                            preferred_element_type=f32)
        sref[z, :, pl.ds(j * w, w)] = t
        lt = _lane_tiles(t)
        mm = lt[0]
        for x in lt[1:]:
            mm = jnp.maximum(mm, x)
        return mm

    def rowmax(mp):
        return jnp.max(mp, axis=-1, keepdims=True)

    def normalize(o, lp):
        l = jnp.sum(lp, axis=-1, keepdims=True)
        return (o * _recip(l)).astype(bf16)

    def oproj(on, slot, c):
        acc_v[pl.ds(c * R, R), :] += jnp.dot(on, wo_v[slot], preferred_element_type=f32)

    def mods():
        ga = mod_v[0:1, 2 * D:3 * D]
        sb = mod_v[0:1, 3 * D:4 * D]
        cb1 = 1.0 + mod_v[0:1, 4 * D:5 * D]
        gb = mod_v[0:1, 5 * D:6 * D]
        return ga, sb, cb1, gb

    def ln2_piece(i, r0, nr, dst):
        ga, sb, cb1, gb = mods()
        rows = pl.ds(pl.multiple_of(i * RF + r0, 16), nr)
        x2 = x_v[rows, :].astype(f32) + ga * acc_v[rows, :]
        dst[pl.ds(r0, nr), :] = (_ln(x2) * cb1 + sb).astype(bf16)

    def run_chunks(h, t0, t1, st, z0, z1, cfg, total=None, hook=None):
        qpj, finj, opj, order, mj, lsum, wa, ajs = cfg
        ga_ = S // wa
        assert ajs is None or len(ajs) == ga_
        assert finj < G and opj < G and qpj < G
        ratio = G // ga_ if ga_ <= G else None

        def hs(t):
            if t < 0:
                return jnp.maximum(h - 1, 0) & MASK
            return (h + t // N) & MASK

        def exists(t):
            return total is None or t < total

        from_scratch = st is None
        q = {t0 + 1: q_c[...] if from_scratch else st[0]}
        m = {} if from_scratch else {t0: st[1]}
        o_prev = l_prev = None
        mp = o = lp = on = None
        for t in range(t0, t1):
            c = t % N
            look = exists(t + 1)
            has_prev = t > t0 or from_scratch or st[2] is not None
            for j in range(G):
                if hook is not None:
                    hook(t, j)

                def stage_a():
                    nonlocal mp
                    if ajs is not None:
                        jas = [i_ for i_, jj in enumerate(ajs) if jj == j]
                    elif ratio is not None:
                        jas = [j // ratio] if j % ratio == 0 else []
                    else:
                        k_ = ga_ // G
                        jas = list(range(j * k_, (j + 1) * k_))
                    for ja in jas:
                        mm = score(q[t + 1], hs(t + 1), ja, wa, s_refs[(c + 1) % 2], z0)
                        mp = mm if ja == 0 else jnp.maximum(mp, mm)
                        if ja == ga_ - 1 and mj == 0:
                            m[t + 1] = rowmax(mp)

                def stage_b():
                    sv = s_refs[c % 2][z1, :, pl.ds(j * W, W)]
                    if t == t0 and from_scratch:
                        if j == 0:
                            m[t] = m_c[...]
                        return jnp.concatenate([jnp.exp2(x - m[t]) for x in _lane_tiles(sv)], axis=1)
                    return jnp.exp2(sv - m[t])

                if qpj < 0 and j == 0 and exists(t + 2):
                    q[t + 2] = qproj(hs(t + 2), (t + 2) % N)
                if opj < 0 and j == 0 and has_prev:
                    if t == t0:
                        o_prev, l_prev = (o_c[...], l_c[...]) if from_scratch else (st[2], st[3])
                    oproj(normalize(o_prev, l_prev), hs(t - 1), (t - 1) % N)
                if look and order == 0:
                    stage_a()
                e = stage_b()
                if look and order == 1:
                    stage_a()
                lt = _lane_tiles(e)
                if lsum == 0:
                    ls = lt[0]
                    for x in lt[1:]:
                        ls = ls + x
                    lp = ls if j == 0 else lp + ls
                else:
                    for i_, x in enumerate(lt):
                        lp = x if (j == 0 and i_ == 0) else lp + x
                def stage_c(tc, jc, pval):
                    nonlocal o
                    vv = v_v[hs(tc), pl.ds(jc * W, W), :]
                    tt = jnp.dot(pval, vv, preferred_element_type=f32)
                    o = tt if jc == 0 else o + tt
                if SK == 0:
                    stage_c(t, j, e.astype(bf16))
                else:
                    p_refs[j % 2][z0] = pltpu.bitcast(e.astype(bf16), jnp.uint32)
                    if j > 0:
                        stage_c(t, j - 1, pltpu.bitcast(p_refs[(j - 1) % 2][z1], bf16))
                    if j == G - 1:
                        stage_c(t, j, pltpu.bitcast(p_refs[j % 2][z1], bf16))
                if look and mj == 1 and j == G - 1:
                    m[t + 1] = rowmax(mp)
                if j == finj and has_prev and opj >= 0:
                    if t == t0:
                        o_prev, l_prev = (o_c[...], l_c[...]) if from_scratch else (st[2], st[3])
                    on = normalize(o_prev, l_prev)
                if j == opj and has_prev:
                    oproj(on, hs(t - 1), (t - 1) % N)
                if j == qpj and exists(t + 2):
                    q[t + 2] = qproj(hs(t + 2), (t + 2) % N)
            o_prev, l_prev = o, lp
        if not exists(t1):
            oproj(normalize(o_prev, l_prev), hs(t1 - 1), (t1 - 1) % N)
            return None
        return (q[t1 + 1], m[t1], o_prev, l_prev)

    def save_state(st):
        q_c[...] = st[0]
        m_c[...] = jnp.broadcast_to(st[1], (R, 128))
        o_c[...] = st[2]
        l_c[...] = st[3]

    hc0 = head_copies(0, 0)
    named = {'c': [cp_c], 'wm0': [cp_wm0], 'wq0': [hc0[0]], 'k0': [hc0[1]], 'v0': [hc0[2]], 'wo0': [hc0[3]],
             'h1': head_copies(1, 1) + head_copies(2, 2), 'xr': cp_x[3:] if _env('DORD', 2) < 8 else cp_x[4:]}
    for i in range(XC):
        named['x%d' % i] = [cp_x[i]]
    stages = {
        0: ['c wm0 x0 wq0 k0 x1 v0 x2 wo0', '', 'xr', '', '', 'h1', '', ''],
        1: ['c wm0 x0', 'wq0 k0', 'x1 v0', '', 'x2 wo0', 'xr', 'h1', ''],
        2: ['c wm0 x0 wq0 k0', '', 'x1 v0', '', 'x2 wo0', 'xr', 'h1', ''],
        3: ['c wm0', 'x0 wq0', 'k0 x1', 'v0', 'x2 wo0', 'xr', 'h1', ''],
        4: ['c wm0 x0', 'wq0 k0', 'x1 v0 x2 wo0', '', 'xr', '', 'h1', ''],
        5: ['c wm0 x0', 'wq0 k0', 'x1 v0', '', 'x2 wo0', 'xr', '', 'h1'],
        6: ['wm0 c x0 wq0', 'k0', 'x1 v0', '', 'x2 wo0', 'xr', '', 'h1'],
        7: ['c wm0 x0 wq0 k0', '', 'x1 v0 x2 wo0', '', '', 'xr', '', 'h1'],
        11: ['c wm0 x0 x1', 'x2 x3 wq0 k0', 'xr', 'v0', 'wo0', '', 'h1', ''],
        12: ['c wm0 x0 x1 x2 x3', 'wq0 k0', 'xr', 'v0', 'wo0', '', 'h1', ''],
        13: ['c wm0 x0 x1', 'x2 x3 wq0', 'k0 xr', 'v0 wo0', '', '', 'h1', ''],
        8: ['c wm0 x0 x1 wq0 k0', '', 'x2 x3 v0', '', 'wo0', 'xr', 'h1', ''],
        9: ['c wm0 x0 x1', 'wq0 k0', 'x2 x3 v0', '', 'wo0', 'xr', 'h1', ''],
        10: ['c wm0 x0 x1 wq0', 'k0', 'x2 x3', '', 'v0 wo0', 'xr', '', 'h1'],
    }[_env("DORD", 2)]
    assert sorted(' '.join(stages).split()) == sorted(('c wm0 x0 wq0 k0 x1 v0 x2 wo0 xr h1' + (' x3' if _env('DORD', 2) >= 8 else '')).split())

    def stage(k):
        for n_ in stages[k].split():
            for cp in named[n_]:
                cp.start()

    stage(0)

    zz = lax.fori_loop(0, 2, lambda i, c: c + lax.shift_right_logical(i, 6), 0)
    za, zb = zz, lax.shift_right_logical(zz, 1)

    scope('prologue')
    acc_v[...] = jnp.zeros_like(acc_v)
    fscope('w_c')
    cp_c.wait()
    fscope('p1')
    stage(1)
    cval = c_v[...].astype(f32)
    sc_v[...] = jnp.broadcast_to((cval * jax.nn.sigmoid(cval)).astype(bf16), (16, D))
    fscope('w_wm0')
    cp_wm0.wait()
    stage(2)
    if PJ:
        x_wait((R - 1) // XR)
        stage(3)
        hc0[0].wait()
        stage(4)
    fscope('mod')
    mod_v[:, pl.ds(0, 2 * D)] = jnp.dot(sc_v[...], wm_v[:, pl.ds(0, 2 * D)], preferred_element_type=f32)
    if not PJ:
        x_wait((R - 1) // XR)
        stage(3)
    ln1(0)
    if not PJ:
        hc0[0].wait()
        stage(4)
    q0 = qproj(0, 0)
    fscope('w_k0')
    hc0[1].wait()
    stage(5)
    fscope('w_x1')
    FXJ = _env("FXJ", 0)
    if FXJ == 0:
        x_wait((2 * R - 1) // XR)
    scope('fill')
    mp0 = None
    for j in range(G):
        mm0 = score(q0, 0, j, W, s0_v, za)
        mp0 = mm0 if j == 0 else jnp.maximum(mp0, mm0)
        if j == FXJ:
            x_wait((2 * R - 1) // XR)
            ln1(1)
    m0 = rowmax(mp0)
    q1 = qproj(0, 1)
    scope('first')

    XWP = [int(v) for v in _E.get("XWP", "0,1" if R == 256 else "0,2,6").split(',')]

    def first_hook(t, j):
        if j == 0:
            if t == 0:
                fscope('w_v0')
                hc0[2].wait()
                hc0[3].wait()
            if t in XWP:
                later = [p_ for p_ in XWP if p_ > t]
                upto_t = later[0] - 1 if later else N - 3
                x_wait(((upto_t + 2) * R + R - 1) // XR)
            if t == 0:
                stage(6)
                fscope('first0')
            if t == 1:
                stage(7)
                fscope('first1')
        if j == L1J and t + 2 < N:
            ln1(t + 2)

    assert RHO >= N - 2 and (RHO + N + 1) // N == 1
    if RHO == 0:
        first_hook(0, 0)
        first_hook(1, 0)
        save_state((q1, m0, jnp.zeros((R, DH), f32), jnp.ones((R, 128), f32)))
    elif ONLY in ('', 'F'):
        save_state(run_chunks(0, 0, RHO, (q1, m0, None, None), za, zb, CFG_F, hook=first_hook))
    scope(None)

    def head_body(h, carry):
        scope('head')
        for cp in head_copies(h + 1, (h + 1) & MASK):
            cp.wait()

        @pl.when(h == 0)
        def _():
            cp_wm1.start()
            cp_wg.start()
            cp_wu.start()
            cp_wd.start()

        z0 = lax.shift_right_logical(h, 6)
        z1 = lax.shift_right_logical(h, 7)
        save_state(run_chunks(h, RHO, RHO + N, None, z0, z1, CFG_L))

        @pl.when(h + 3 < H)
        def _():
            for cp in head_copies(jnp.minimum(h + 3, H - 1), (h + 3) & MASK):
                cp.start()

        scope(None)
        return carry

    if _env("NODMA", 0) == 1:
        for cp in head_copies(1, 1):
            cp.wait()
    if ONLY in ('', 'L'):
        lax.fori_loop(0, H - 1, head_body, 0)

    def out_copy(i):
        rows = pl.ds(pl.multiple_of(i * RF, RF), RF)
        return pltpu.make_async_copy(out_v.at[rows, :], o_hbm.at[rows, :], sem_out.at[i])

    scope('last')
    cp_wm1.wait()
    cp_wg.wait()
    cp_wu.wait()
    cp_wd.wait()
    mod_v[:, pl.ds(2 * D, 4 * D)] = jnp.dot(sc_v[...], wm_v[:, pl.ds(2 * D, 4 * D)], preferred_element_type=f32)

    def last_hook(t, j):
        if t == min(L2T, N - 1) and j == (L2J if L2T < N else G - 1):
            ln2_piece(0, 0, RF, h2_v.at[za] if MERGE else h2_v.at[0])

    L2T = max(RHO, (RF - 1) // R + 2)
    assert L2T < N or RHO == 0
    if ONLY in ('', 'E'):
        run_chunks(H - 1, RHO, N, None, za, zb, CFG_E, total=N, hook=last_hook)

    def ffn_chunk(i, src, dst):
        ga, sb, cb1, gb = mods()
        nxt = jnp.minimum(i + 1, NF - 1) if not isinstance(i, int) else min(i + 1, NF - 1)
        y = None
        pr = RF // LNP
        for j in range(NG):
            cols = pl.ds(j * FW, FW)
            h2 = src[...]
            g = jnp.dot(h2, wg_v[:, cols], preferred_element_type=f32)
            u = jnp.dot(h2, wu_v[:, cols], preferred_element_type=f32)
            a = (jax.nn.gelu(g, approximate=True) * u).astype(bf16)
            t = jnp.dot(a, wd_v[cols, :], preferred_element_type=f32)
            y = t if j == 0 else y + t
            if LN0 <= j < LN0 + LNP:
                ln2_piece(nxt, (j - LN0) * pr, pr, dst)
        rows = pl.ds(pl.multiple_of(i * RF, RF), RF)
        x2 = x_v[rows, :].astype(f32) + ga * acc_v[rows, :]
        out_v[rows, :] = (x2 + gb * y).astype(bf16)
        out_copy(i).start()

    def ffn_body(i, carry):
        scope('ffn')
        ffn_chunk(i, h2_v.at[i & 1], h2_v.at[(i + 1) & 1])
        scope(None)
        return carry

    if MERGE:
        ffn_chunk(0, h2_v.at[zb], h2_v.at[1])
    scope(None)
    if ONLY in ('', 'N'):
        lax.fori_loop(MERGE, NF, ffn_body, 0)
    scope('tail')
    for i in range(NF):
        out_copy(i).wait()
    scope(None)


@jax.jit
def pallas_adaLN_cond__mha_block_cached__geglu_ffn__prompt_kernel(
        A_x, A_k_cache, A_v_cache, A_wq, A_wo, B_x, B_w_gate, B_w_up, B_w_down, c, w_mod):
    del B_x
    x = A_x.reshape(S, D)
    k = A_k_cache.reshape(H, S, DH)
    v = A_v_cache.reshape(H, S, DH)
    anyspec = pl.BlockSpec(memory_space=pl.ANY)
    out = pl.pallas_call(
        _kernel,
        in_specs=[anyspec] * 10,
        out_specs=anyspec,
        out_shape=jax.ShapeDtypeStruct((S, D), bf16),
        scratch_shapes=[
            pltpu.VMEM((S, D), bf16),
            pltpu.VMEM((NSLOT, S, DH), bf16),
            pltpu.VMEM((NSLOT, S, DH), bf16),
            pltpu.VMEM((NSLOT, D, DH), bf16),
            pltpu.VMEM((NSLOT, DH, D), bf16),
            pltpu.VMEM((D, F), bf16),
            pltpu.VMEM((D, F), bf16),
            pltpu.VMEM((F, D), bf16),
            pltpu.VMEM((1, D), bf16),
            pltpu.VMEM((D, 6 * D), bf16),
            pltpu.VMEM((S, D), bf16),
            pltpu.VMEM((16, 6 * D), f32),
            pltpu.VMEM((16, D), bf16),
            pltpu.VMEM((D // 128, S, 128) if U32 & 8 else (S, D), bf16),
            pltpu.VMEM((S, D), f32),
            pltpu.VMEM((2, R, S), f32),
            pltpu.VMEM((2, R, S), f32),
            pltpu.VMEM((R, 128), f32),
            pltpu.VMEM((R, DH), bf16),
            pltpu.VMEM((R, DH), f32),
            pltpu.VMEM((R, 128), f32),
            pltpu.VMEM((2, RF, D), bf16),
            pltpu.VMEM((2, R // 2, W), jnp.uint32),
            pltpu.VMEM((2, R // 2, W), jnp.uint32),
            pltpu.SemaphoreType.DMA((4, NSLOT)),
            pltpu.SemaphoreType.DMA((6,)),
            pltpu.SemaphoreType.DMA((XC,)),
            pltpu.SemaphoreType.DMA((NF,)),
        ],
        compiler_params=pltpu.CompilerParams(
            vmem_limit_bytes=100 * 1024 * 1024,
            disable_bounds_checks=bool(_env("NOBC", 1)),
            disable_semaphore_checks=bool(_env("NOSC", 1)),
            flags={"XLA_TPU_FORCE_LP_LLO_SCHEDULER": True} if LP else {},
        ),
    )(x, k, v, A_wq, A_wo, B_w_gate, B_w_up, B_w_down, c, w_mod)
    return out.reshape(1, S, D)
```

```python
import jax
import jax.numpy as jnp
from jax import lax
import jax.experimental.pallas as pl
import jax.experimental.pallas.tpu as pltpu

H, DH, S, D, F = 32, 128, 2048, 512, 1792
R = 512
W = 512
N = S // R
G = S // W
RHO = 2
NSLOT = 4
RF = 256
FW = 256
NF = S // RF
XR = 256
XC = S // XR
EPS = 1e-5
LOG2E = 1.4426950408889634

SCHED_LOOP = dict(a=2, q=-1, n=1, o=2)
SCHED_EDGE = dict(a=0, q=0, n=1, o=2)

f32 = jnp.float32
bf16 = jnp.bfloat16


def _lane_tiles(x):
    return [x[:, i * 128:(i + 1) * 128] for i in range(x.shape[1] // 128)]


def _layernorm(x):
    m = jnp.mean(x, axis=-1, keepdims=True)
    xc = x - m
    v = jnp.mean(xc * xc, axis=-1, keepdims=True)
    return xc * lax.rsqrt(v + EPS)


def _reciprocal(l):
    r = pl.reciprocal(l, approx=True)
    return r * (2.0 - l * r)


def _kernel(x_hbm, k_hbm, v_hbm, wq_hbm, wo_hbm, wg_hbm, wu_hbm, wd_hbm, c_hbm, wm_hbm, o_hbm,
            x_v, k_v, v_v, wq_v, wo_v, wg_v, wu_v, wd_v, c_v, wm_v, out_v,
            mod_v, sc_v, h_v, acc_v, s0_v, s1_v, m_c, q_c, o_c, l_c, h2_v,
            sem_head, sem_misc, sem_x, sem_out):
    scale = (DH ** -0.5) * LOG2E
    s_refs = (s0_v, s1_v)

    def head_copies(h, slot):
        col = pl.multiple_of(h * DH, DH)
        return [
            pltpu.make_async_copy(wq_hbm.at[:, pl.ds(col, DH)], wq_v.at[slot], sem_head.at[0, slot]),
            pltpu.make_async_copy(k_hbm.at[h], k_v.at[slot], sem_head.at[1, slot]),
            pltpu.make_async_copy(v_hbm.at[h], v_v.at[slot], sem_head.at[2, slot]),
            pltpu.make_async_copy(wo_hbm.at[h], wo_v.at[slot], sem_head.at[3, slot]),
        ]

    cp_c = pltpu.make_async_copy(c_hbm, c_v, sem_misc.at[0])
    cp_wm0 = pltpu.make_async_copy(wm_hbm.at[:, pl.ds(0, 2 * D)], wm_v.at[:, pl.ds(0, 2 * D)], sem_misc.at[1])
    cp_wm1 = pltpu.make_async_copy(wm_hbm.at[:, pl.ds(2 * D, 4 * D)], wm_v.at[:, pl.ds(2 * D, 4 * D)],
                                   sem_misc.at[2])
    cp_ffn = [cp_wm1,
              pltpu.make_async_copy(wg_hbm, wg_v, sem_misc.at[3]),
              pltpu.make_async_copy(wu_hbm, wu_v, sem_misc.at[4]),
              pltpu.make_async_copy(wd_hbm, wd_v, sem_misc.at[5])]
    cp_x = [pltpu.make_async_copy(x_hbm.at[pl.ds(i * XR, XR), :], x_v.at[pl.ds(i * XR, XR), :], sem_x.at[i])
            for i in range(XC)]

    def out_copy(i):
        rows = pl.ds(pl.multiple_of(i * RF, RF), RF)
        return pltpu.make_async_copy(out_v.at[rows, :], o_hbm.at[rows, :], sem_out.at[i])

    def ln1(c):
        sa = mod_v[0:1, 0:D]
        ca1 = 1.0 + mod_v[0:1, D:2 * D]
        rows = pl.ds(c * R, R)
        h_v[rows, :] = (_layernorm(x_v[rows, :].astype(f32)) * ca1 + sa).astype(bf16)

    def ffn_mods():
        ga = mod_v[0:1, 2 * D:3 * D]
        sb = mod_v[0:1, 3 * D:4 * D]
        cb1 = 1.0 + mod_v[0:1, 4 * D:5 * D]
        gb = mod_v[0:1, 5 * D:6 * D]
        return ga, sb, cb1, gb

    def ln2(i, r0, nr, dst):
        ga, sb, cb1, _ = ffn_mods()
        rows = pl.ds(pl.multiple_of(i * RF + r0, 16), nr)
        x2 = x_v[rows, :].astype(f32) + ga * acc_v[rows, :]
        dst[pl.ds(r0, nr), :] = (_layernorm(x2) * cb1 + sb).astype(bf16)

    class Heads:
        def __init__(self, h0, c0):
            self.h0, self.c0, self.cache = h0, c0, {}

        def views(self, t):
            dh = (self.c0 + t) // N
            if dh not in self.cache:
                slot = (self.h0 + dh) & (NSLOT - 1)
                self.cache[dh] = dict(k=k_v.at[slot], v=v_v.at[slot], wq=wq_v.at[slot], wo=wo_v.at[slot])
            return self.cache[dh]

        def rows(self, t):
            return pl.ds(((self.c0 + t) % N) * R, R)

    def qproj(hd, t):
        q = jnp.dot(h_v[hd.rows(t), :], hd.views(t)['wq'][...], preferred_element_type=f32)
        return (q * scale).astype(bf16)

    def scores(q, hd, t, k0, nk, sref, z):
        s = lax.dot_general(q, hd.views(t)['k'][pl.ds(k0, nk), :], (((1,), (1,)), ((), ())),
                            preferred_element_type=f32)
        sref[z, :, pl.ds(k0, nk)] = s
        lt = _lane_tiles(s)
        mm = lt[0]
        for x in lt[1:]:
            mm = jnp.maximum(mm, x)
        return mm

    def rowmax(mp):
        return jnp.max(mp, axis=-1, keepdims=True)

    def normalize(o, lp):
        l = jnp.sum(lp, axis=-1, keepdims=True)
        return (o * _reciprocal(l)).astype(bf16)

    def oproj(on, hd, t):
        acc_v[hd.rows(t), :] += jnp.dot(on, hd.views(t)['wo'][...], preferred_element_type=f32)

    def run_positions(hd, n, st, z0, z1, sched, last=False, hook=None):
        def exists(t):
            return not last or t < n

        from_scratch = st is None
        q = {1: q_c[...] if from_scratch else st[0]}
        m = {} if from_scratch else {0: st[1]}
        o_prev = l_prev = o = lp = on = None
        for t in range(n):
            has_prev = t > 0 or from_scratch or st[2] is not None
            for j in range(G):
                if hook is not None:
                    hook(t, j)
                if sched['q'] < 0 and j == 0 and exists(t + 2):
                    q[t + 2] = qproj(hd, t + 2)
                if j == sched['a'] and exists(t + 1):
                    m[t + 1] = rowmax(scores(q[t + 1], hd, t + 1, 0, S, s_refs[(t + 1) % 2], z0))
                sv = s_refs[t % 2][z1, :, pl.ds(j * W, W)]
                if t == 0 and from_scratch:
                    if j == 0:
                        m[0] = m_c[...]
                    e = jnp.concatenate([jnp.exp2(x - m[0]) for x in _lane_tiles(sv)], axis=1)
                else:
                    e = jnp.exp2(sv - m[t])
                for i, x in enumerate(_lane_tiles(e)):
                    lp = x if (j == 0 and i == 0) else lp + x
                pv = jnp.dot(e.astype(bf16), hd.views(t)['v'][pl.ds(j * W, W), :], preferred_element_type=f32)
                o = pv if j == 0 else o + pv
                if j == sched['n'] and has_prev:
                    if t == 0:
                        o_prev, l_prev = (o_c[...], l_c[...]) if from_scratch else (st[2], st[3])
                    on = normalize(o_prev, l_prev)
                if j == sched['o'] and has_prev:
                    oproj(on, hd, t - 1)
                if j == sched['q'] and exists(t + 2):
                    q[t + 2] = qproj(hd, t + 2)
            o_prev, l_prev = o, lp
        if last:
            oproj(normalize(o_prev, l_prev), hd, n - 1)
            return None
        return q[n + 1], m[n], o_prev, l_prev

    def save_state(st):
        q_c[...] = st[0]
        m_c[...] = jnp.broadcast_to(st[1], (R, 128))
        o_c[...] = st[2]
        l_c[...] = st[3]

    cp_wq0, cp_k0, cp_v0, cp_wo0 = head_copies(0, 0)
    for cp in (cp_c, cp_wm0, cp_x[0], cp_x[1], cp_wq0, cp_k0):
        cp.start()

    za = lax.fori_loop(0, 2, lambda i, c: c + lax.shift_right_logical(i, 6), 0)
    zb = lax.shift_right_logical(za, 1)

    acc_v[...] = jnp.zeros_like(acc_v)
    cp_c.wait()
    cval = c_v[...].astype(f32)
    sc_v[...] = jnp.broadcast_to((cval * jax.nn.sigmoid(cval)).astype(bf16), (16, D))
    cp_wm0.wait()
    for cp in (cp_x[2], cp_x[3], cp_v0):
        cp.start()
    cp_x[0].wait()
    cp_x[1].wait()
    cp_wq0.wait()
    cp_wo0.start()
    mod_v[:, pl.ds(0, 2 * D)] = jnp.dot(sc_v[...], wm_v[:, pl.ds(0, 2 * D)], preferred_element_type=f32)
    ln1(0)
    head0 = Heads(0, 0)
    q0 = qproj(head0, 0)
    cp_k0.wait()
    for cp in cp_x[4:]:
        cp.start()

    mp0 = None
    for j in range(G):
        mm0 = scores(q0, head0, 0, j * W, W, s0_v, za)
        mp0 = mm0 if j == 0 else jnp.maximum(mp0, mm0)
        if j == 1:
            cp_x[2].wait()
            cp_x[3].wait()
            ln1(1)
    m0 = rowmax(mp0)
    q1 = qproj(head0, 1)

    def first_hook(t, j):
        if j == 0:
            if t == 0:
                cp_v0.wait()
                cp_wo0.wait()
            cp_x[4 + 2 * t].wait()
            cp_x[5 + 2 * t].wait()
            if t == 0:
                for cp in head_copies(1, 1) + head_copies(2, 2):
                    cp.start()
            ln1(t + 2)

    save_state(run_positions(head0, RHO, (q1, m0, None, None), za, zb, SCHED_EDGE, hook=first_hook))

    def head_body(h, carry):
        for cp in head_copies(h + 1, (h + 1) & (NSLOT - 1)):
            cp.wait()

        @pl.when(h == 0)
        def _():
            for cp in cp_ffn:
                cp.start()

        z0 = lax.shift_right_logical(h, 6)
        z1 = lax.shift_right_logical(h, 7)
        save_state(run_positions(Heads(h, RHO), N, None, z0, z1, SCHED_LOOP))
        h3 = h + 3

        @pl.when(h3 < H)
        def _():
            for cp in head_copies(jnp.minimum(h3, H - 1), h3 & (NSLOT - 1)):
                cp.start()

        return carry

    lax.fori_loop(0, H - 1, head_body, 0)

    for cp in cp_ffn:
        cp.wait()
    mod_v[:, pl.ds(2 * D, 4 * D)] = jnp.dot(sc_v[...], wm_v[:, pl.ds(2 * D, 4 * D)], preferred_element_type=f32)

    def last_hook(t, j):
        if t == 0 and j == 0:
            ln2(0, 0, RF, h2_v.at[0])

    run_positions(Heads(H - 1, RHO), N - RHO, None, za, zb, SCHED_EDGE, last=True, hook=last_hook)

    def ffn_body(i, carry):
        ga, _, _, gb = ffn_mods()
        src = h2_v.at[i & 1]
        dst = h2_v.at[(i + 1) & 1]
        nxt = jnp.minimum(i + 1, NF - 1)
        y = None
        for j in range(F // FW):
            cols = pl.ds(j * FW, FW)
            h2 = src[...]
            g = jnp.dot(h2, wg_v[:, cols], preferred_element_type=f32)
            u = jnp.dot(h2, wu_v[:, cols], preferred_element_type=f32)
            a = (jax.nn.gelu(g, approximate=True) * u).astype(bf16)
            t = jnp.dot(a, wd_v[cols, :], preferred_element_type=f32)
            y = t if j == 0 else y + t
            if j in (2, 3):
                ln2(nxt, (j - 2) * (RF // 2), RF // 2, dst)
        rows = pl.ds(pl.multiple_of(i * RF, RF), RF)
        x2 = x_v[rows, :].astype(f32) + ga * acc_v[rows, :]
        out_v[rows, :] = (x2 + gb * y).astype(bf16)
        out_copy(i).start()
        return carry

    lax.fori_loop(0, NF, ffn_body, 0)
    for i in range(NF):
        out_copy(i).wait()


@jax.jit
def pallas_adaLN_cond__mha_block_cached__geglu_ffn__prompt_kernel(
    A_x: jax.Array,
    A_k_cache: jax.Array,
    A_v_cache: jax.Array,
    A_wq: jax.Array,
    A_wo: jax.Array,
    B_x: jax.Array,
    B_w_gate: jax.Array,
    B_w_up: jax.Array,
    B_w_down: jax.Array,
    c: jax.Array,
    w_mod: jax.Array,
):
    del B_x
    hbm = pl.BlockSpec(memory_space=pl.ANY)
    out = pl.pallas_call(
        _kernel,
        in_specs=[hbm] * 10,
        out_specs=hbm,
        out_shape=jax.ShapeDtypeStruct((S, D), bf16),
        scratch_shapes=[
            pltpu.VMEM((S, D), bf16),
            pltpu.VMEM((NSLOT, S, DH), bf16),
            pltpu.VMEM((NSLOT, S, DH), bf16),
            pltpu.VMEM((NSLOT, D, DH), bf16),
            pltpu.VMEM((NSLOT, DH, D), bf16),
            pltpu.VMEM((D, F), bf16),
            pltpu.VMEM((D, F), bf16),
            pltpu.VMEM((F, D), bf16),
            pltpu.VMEM((1, D), bf16),
            pltpu.VMEM((D, 6 * D), bf16),
            pltpu.VMEM((S, D), bf16),
            pltpu.VMEM((16, 6 * D), f32),
            pltpu.VMEM((16, D), bf16),
            pltpu.VMEM((S, D), bf16),
            pltpu.VMEM((S, D), f32),
            pltpu.VMEM((2, R, S), f32),
            pltpu.VMEM((2, R, S), f32),
            pltpu.VMEM((R, 128), f32),
            pltpu.VMEM((R, DH), bf16),
            pltpu.VMEM((R, DH), f32),
            pltpu.VMEM((R, 128), f32),
            pltpu.VMEM((2, RF, D), bf16),
            pltpu.SemaphoreType.DMA((4, NSLOT)),
            pltpu.SemaphoreType.DMA((6,)),
            pltpu.SemaphoreType.DMA((XC,)),
            pltpu.SemaphoreType.DMA((NF,)),
        ],
        compiler_params=pltpu.CompilerParams(
            vmem_limit_bytes=100 * 1024 * 1024,
            disable_bounds_checks=True,
            disable_semaphore_checks=True,
            flags={"XLA_TPU_FORCE_LP_LLO_SCHEDULER": True},
        ),
    )(
        A_x.reshape(S, D),
        A_k_cache.reshape(H, S, DH),
        A_v_cache.reshape(H, S, DH),
        A_wq,
        A_wo.reshape(H, DH, D),
        B_w_gate,
        B_w_up,
        B_w_down,
        c,
        w_mod,
    )
    return out.reshape(1, S, D)
```

```python
import jax
import jax.numpy as jnp
from jax import lax
import jax.experimental.pallas as pl
import jax.experimental.pallas.tpu as pltpu

H, DH, S, D, F = 32, 128, 2048, 512, 1792
R = 512
W = 512
N = S // R
G = S // W
RHO = 2
NSLOT = 4
RF = 256
FW = 256
NF = S // RF
XR = 256
XC = S // XR
EPS = 1e-5
LOG2E = 1.4426950408889634

SCHED_LOOP = dict(q=-1, a=2, n=1, o=2)
SCHED_EDGE = dict(q=-1, a=1, n=1, o=2)

f32 = jnp.float32
bf16 = jnp.bfloat16


def _lane_tiles(x):
    return [x[:, i * 128:(i + 1) * 128] for i in range(x.shape[1] // 128)]


def _layernorm(x):
    m = jnp.mean(x, axis=-1, keepdims=True)
    xc = x - m
    v = jnp.mean(xc * xc, axis=-1, keepdims=True)
    return xc * lax.rsqrt(v + EPS)


def _reciprocal(l):
    r = pl.reciprocal(l, approx=True)
    return r * (2.0 - l * r)


def _kernel(x_hbm, k_hbm, v_hbm, wq_hbm, wo_hbm, wg_hbm, wu_hbm, wd_hbm, c_hbm, wm_hbm, o_hbm,
            x_v, k_v, v_v, wq_v, wo_v, wg_v, wu_v, wd_v, c_v, wm_v, out_v,
            mod_v, sc_v, h_v, acc_v, s0_v, s1_v, m_c, o_c, l_c, h2_v,
            sem_head, sem_misc, sem_x, sem_out):
    scale = (DH ** -0.5) * LOG2E
    s_refs = (s0_v, s1_v)

    def head_copies(h, slot):
        col = pl.multiple_of(h * DH, DH)
        return [
            pltpu.make_async_copy(wq_hbm.at[:, pl.ds(col, DH)], wq_v.at[slot], sem_head.at[0, slot]),
            pltpu.make_async_copy(k_hbm.at[h], k_v.at[slot], sem_head.at[1, slot]),
            pltpu.make_async_copy(v_hbm.at[h], v_v.at[slot], sem_head.at[2, slot]),
            pltpu.make_async_copy(wo_hbm.at[h], wo_v.at[slot], sem_head.at[3, slot]),
        ]

    cp_c = pltpu.make_async_copy(c_hbm, c_v, sem_misc.at[0])
    cp_wm0 = pltpu.make_async_copy(wm_hbm.at[:, pl.ds(0, 2 * D)], wm_v.at[:, pl.ds(0, 2 * D)], sem_misc.at[1])
    cp_wm1 = pltpu.make_async_copy(wm_hbm.at[:, pl.ds(2 * D, 4 * D)], wm_v.at[:, pl.ds(2 * D, 4 * D)],
                                   sem_misc.at[2])
    cp_ffn = [cp_wm1,
              pltpu.make_async_copy(wg_hbm, wg_v, sem_misc.at[3]),
              pltpu.make_async_copy(wu_hbm, wu_v, sem_misc.at[4]),
              pltpu.make_async_copy(wd_hbm, wd_v, sem_misc.at[5])]
    cp_x = [pltpu.make_async_copy(x_hbm.at[pl.ds(i * XR, XR), :], x_v.at[pl.ds(i * XR, XR), :], sem_x.at[i])
            for i in range(XC)]

    def out_copy(i):
        rows = pl.ds(pl.multiple_of(i * RF, RF), RF)
        return pltpu.make_async_copy(out_v.at[rows, :], o_hbm.at[rows, :], sem_out.at[i])

    def ln1(c):
        sa = mod_v[0:1, 0:D]
        ca1 = 1.0 + mod_v[0:1, D:2 * D]
        rows = pl.ds(c * R, R)
        h_v[rows, :] = (_layernorm(x_v[rows, :].astype(f32)) * ca1 + sa).astype(bf16)

    def ffn_mods():
        ga = mod_v[0:1, 2 * D:3 * D]
        sb = mod_v[0:1, 3 * D:4 * D]
        cb1 = 1.0 + mod_v[0:1, 4 * D:5 * D]
        gb = mod_v[0:1, 5 * D:6 * D]
        return ga, sb, cb1, gb

    def ln2(i, r0, nr, dst):
        ga, sb, cb1, _ = ffn_mods()
        rows = pl.ds(pl.multiple_of(i * RF + r0, 16), nr)
        x2 = x_v[rows, :].astype(f32) + ga * acc_v[rows, :]
        dst[pl.ds(r0, nr), :] = (_layernorm(x2) * cb1 + sb).astype(bf16)

    class Heads:
        def __init__(self, h0, c0):
            self.h0, self.c0, self.cache = h0, c0, {}

        def views(self, t):
            dh = (self.c0 + t) // N
            if dh not in self.cache:
                slot = (self.h0 + dh) & (NSLOT - 1)
                self.cache[dh] = dict(k=k_v.at[slot], v=v_v.at[slot], wq=wq_v.at[slot], wo=wo_v.at[slot])
            return self.cache[dh]

        def rows(self, t):
            return pl.ds(((self.c0 + t) % N) * R, R)

    def qproj(hd, t):
        q = jnp.dot(h_v[hd.rows(t), :], hd.views(t)['wq'][...], preferred_element_type=f32)
        return (q * scale).astype(bf16)

    def scores(q, hd, t, k0, nk, sref, z):
        s = lax.dot_general(q, hd.views(t)['k'][pl.ds(k0, nk), :], (((1,), (1,)), ((), ())),
                            preferred_element_type=f32)
        sref[z, :, pl.ds(k0, nk)] = s
        lt = _lane_tiles(s)
        mm = lt[0]
        for x in lt[1:]:
            mm = jnp.maximum(mm, x)
        return mm

    def rowmax(mp):
        return jnp.max(mp, axis=-1, keepdims=True)

    def normalize(o, lp):
        l = jnp.sum(lp, axis=-1, keepdims=True)
        return (o * _reciprocal(l)).astype(bf16)

    def oproj(on, hd, t):
        acc_v[hd.rows(t), :] += jnp.dot(on, hd.views(t)['wo'][...], preferred_element_type=f32)

    def run_positions(hd, n, st, z0, z1, sched, last=False, hook=None):
        def exists(t):
            return not last or t < n

        from_scratch = st is None
        m = {} if from_scratch else {0: st[0]}
        o_prev = l_prev = o = lp = on = q = None
        assert sched['q'] < sched['a']
        for t in range(n):
            has_prev = t > 0 or from_scratch or st[1] is not None
            for j in range(G):
                if hook is not None:
                    hook(t, j)
                if sched['q'] < 0 and j == 0 and exists(t + 1):
                    q = qproj(hd, t + 1)
                if j == sched['a'] and exists(t + 1):
                    m[t + 1] = rowmax(scores(q, hd, t + 1, 0, S, s_refs[(t + 1) % 2], z0))
                sv = s_refs[t % 2][z1, :, pl.ds(j * W, W)]
                if t == 0 and from_scratch:
                    if j == 0:
                        m[0] = m_c[...]
                    e = jnp.concatenate([jnp.exp2(x - m[0]) for x in _lane_tiles(sv)], axis=1)
                else:
                    e = jnp.exp2(sv - m[t])
                for i, x in enumerate(_lane_tiles(e)):
                    lp = x if (j == 0 and i == 0) else lp + x
                pv = jnp.dot(e.astype(bf16), hd.views(t)['v'][pl.ds(j * W, W), :], preferred_element_type=f32)
                o = pv if j == 0 else o + pv
                if j == sched['n'] and has_prev:
                    if t == 0:
                        o_prev, l_prev = (o_c[...], l_c[...]) if from_scratch else (st[1], st[2])
                    on = normalize(o_prev, l_prev)
                if j == sched['o'] and has_prev:
                    oproj(on, hd, t - 1)
                if j == sched['q'] and exists(t + 1):
                    q = qproj(hd, t + 1)
            o_prev, l_prev = o, lp
        if last:
            oproj(normalize(o_prev, l_prev), hd, n - 1)
            return None
        return m[n], o_prev, l_prev

    def save_state(st):
        m_c[...] = jnp.broadcast_to(st[0], (R, 128))
        o_c[...] = st[1]
        l_c[...] = st[2]

    cp_wq0, cp_k0, cp_v0, cp_wo0 = head_copies(0, 0)
    for cp in (cp_c, cp_wm0, cp_x[0], cp_x[1], cp_wq0, cp_k0):
        cp.start()

    za = lax.fori_loop(0, 2, lambda i, c: c + lax.shift_right_logical(i, 6), 0)
    zb = lax.shift_right_logical(za, 1)

    acc_v[...] = jnp.zeros_like(acc_v)
    cp_c.wait()
    cval = c_v[...].astype(f32)
    sc_v[...] = jnp.broadcast_to((cval * jax.nn.sigmoid(cval)).astype(bf16), (16, D))
    cp_wm0.wait()
    for cp in (cp_x[2], cp_x[3], cp_v0):
        cp.start()
    cp_x[0].wait()
    cp_x[1].wait()
    cp_wq0.wait()
    cp_wo0.start()
    mod_v[:, pl.ds(0, 2 * D)] = jnp.dot(sc_v[...], wm_v[:, pl.ds(0, 2 * D)], preferred_element_type=f32)
    ln1(0)
    head0 = Heads(0, 0)
    q0 = qproj(head0, 0)
    cp_k0.wait()
    for cp in cp_x[4:]:
        cp.start()

    mp0 = None
    for j in range(G):
        mm0 = scores(q0, head0, 0, j * W, W, s0_v, za)
        mp0 = mm0 if j == 0 else jnp.maximum(mp0, mm0)
        if j == 1:
            cp_x[2].wait()
            cp_x[3].wait()
            ln1(1)
    m0 = rowmax(mp0)

    def first_hook(t, j):
        if j == 0:
            if t == 0:
                cp_v0.wait()
                cp_wo0.wait()
            cp_x[4 + 2 * t].wait()
            cp_x[5 + 2 * t].wait()
            if t == 0:
                for cp in head_copies(1, 1) + head_copies(2, 2):
                    cp.start()
            ln1(t + 2)

    save_state(run_positions(head0, RHO, (m0, None, None), za, zb, SCHED_EDGE, hook=first_hook))

    def head_body(h, carry):
        for cp in head_copies(h + 1, (h + 1) & (NSLOT - 1)):
            cp.wait()

        @pl.when(h == 0)
        def _():
            for cp in cp_ffn:
                cp.start()

        z0 = lax.shift_right_logical(h, 6)
        z1 = lax.shift_right_logical(h, 7)
        save_state(run_positions(Heads(h, RHO), N, None, z0, z1, SCHED_LOOP))
        h3 = h + 3

        @pl.when(h3 < H)
        def _():
            for cp in head_copies(jnp.minimum(h3, H - 1), h3 & (NSLOT - 1)):
                cp.start()

        return carry

    lax.fori_loop(0, H - 1, head_body, 0)

    for cp in cp_ffn:
        cp.wait()
    mod_v[:, pl.ds(2 * D, 4 * D)] = jnp.dot(sc_v[...], wm_v[:, pl.ds(2 * D, 4 * D)], preferred_element_type=f32)

    def last_hook(t, j):
        if t == 0 and j == 0:
            ln2(0, 0, RF, h2_v.at[0])

    run_positions(Heads(H - 1, RHO), N - RHO, None, za, zb, SCHED_EDGE, last=True, hook=last_hook)

    def ffn_body(i, carry):
        ga, _, _, gb = ffn_mods()
        src = h2_v.at[i & 1]
        dst = h2_v.at[(i + 1) & 1]
        nxt = jnp.minimum(i + 1, NF - 1)
        y = None
        for j in range(F // FW):
            cols = pl.ds(j * FW, FW)
            h2 = src[...]
            g = jnp.dot(h2, wg_v[:, cols], preferred_element_type=f32)
            u = jnp.dot(h2, wu_v[:, cols], preferred_element_type=f32)
            a = (jax.nn.gelu(g, approximate=True) * u).astype(bf16)
            t = jnp.dot(a, wd_v[cols, :], preferred_element_type=f32)
            y = t if j == 0 else y + t
            if j in (2, 3):
                ln2(nxt, (j - 2) * (RF // 2), RF // 2, dst)
        rows = pl.ds(pl.multiple_of(i * RF, RF), RF)
        x2 = x_v[rows, :].astype(f32) + ga * acc_v[rows, :]
        out_v[rows, :] = (x2 + gb * y).astype(bf16)
        out_copy(i).start()
        return carry

    lax.fori_loop(0, NF, ffn_body, 0)
    for i in range(NF):
        out_copy(i).wait()


@jax.jit
def pallas_adaLN_cond__mha_block_cached__geglu_ffn__prompt_kernel(
    A_x: jax.Array,
    A_k_cache: jax.Array,
    A_v_cache: jax.Array,
    A_wq: jax.Array,
    A_wo: jax.Array,
    B_x: jax.Array,
    B_w_gate: jax.Array,
    B_w_up: jax.Array,
    B_w_down: jax.Array,
    c: jax.Array,
    w_mod: jax.Array,
):
    del B_x
    hbm = pl.BlockSpec(memory_space=pl.ANY)
    out = pl.pallas_call(
        _kernel,
        in_specs=[hbm] * 10,
        out_specs=hbm,
        out_shape=jax.ShapeDtypeStruct((S, D), bf16),
        scratch_shapes=[
            pltpu.VMEM((S, D), bf16),
            pltpu.VMEM((NSLOT, S, DH), bf16),
            pltpu.VMEM((NSLOT, S, DH), bf16),
            pltpu.VMEM((NSLOT, D, DH), bf16),
            pltpu.VMEM((NSLOT, DH, D), bf16),
            pltpu.VMEM((D, F), bf16),
            pltpu.VMEM((D, F), bf16),
            pltpu.VMEM((F, D), bf16),
            pltpu.VMEM((1, D), bf16),
            pltpu.VMEM((D, 6 * D), bf16),
            pltpu.VMEM((S, D), bf16),
            pltpu.VMEM((16, 6 * D), f32),
            pltpu.VMEM((16, D), bf16),
            pltpu.VMEM((S, D), bf16),
            pltpu.VMEM((S, D), f32),
            pltpu.VMEM((2, R, S), f32),
            pltpu.VMEM((2, R, S), f32),
            pltpu.VMEM((R, 128), f32),
            pltpu.VMEM((R, DH), f32),
            pltpu.VMEM((R, 128), f32),
            pltpu.VMEM((2, RF, D), bf16),
            pltpu.SemaphoreType.DMA((4, NSLOT)),
            pltpu.SemaphoreType.DMA((6,)),
            pltpu.SemaphoreType.DMA((XC,)),
            pltpu.SemaphoreType.DMA((NF,)),
        ],
        compiler_params=pltpu.CompilerParams(
            vmem_limit_bytes=100 * 1024 * 1024,
            disable_bounds_checks=True,
            disable_semaphore_checks=True,
            flags={"XLA_TPU_FORCE_LP_LLO_SCHEDULER": True},
        ),
    )(
        A_x.reshape(S, D),
        A_k_cache.reshape(H, S, DH),
        A_v_cache.reshape(H, S, DH),
        A_wq,
        A_wo.reshape(H, DH, D),
        B_w_gate,
        B_w_up,
        B_w_down,
        c,
        w_mod,
    )
    return out.reshape(1, S, D)
```

```python
import jax
import jax.numpy as jnp
from jax import lax
import jax.experimental.pallas as pl
import jax.experimental.pallas.tpu as pltpu

H, DH, S, D, F = 32, 128, 2048, 512, 1792
R = 512
W = 512
N = S // R
G = S // W
RHO = 3
NSLOT = 4
RF = 256
FW = 256
NF = S // RF
XR = 256
XC = S // XR
EPS = 1e-5
LOG2E = 1.4426950408889634

SCHED_LOOP = dict(q=0, a=2, n=1, o=2)
SCHED_EDGE = dict(q=-1, a=1, n=1, o=2)

f32 = jnp.float32
bf16 = jnp.bfloat16


def _lane_tiles(x):
    return [x[:, i * 128:(i + 1) * 128] for i in range(x.shape[1] // 128)]


def _layernorm(x):
    m = jnp.mean(x, axis=-1, keepdims=True)
    xc = x - m
    v = jnp.mean(xc * xc, axis=-1, keepdims=True)
    return xc * lax.rsqrt(v + EPS)


def _reciprocal(l):
    r = pl.reciprocal(l, approx=True)
    return r * (2.0 - l * r)


def _kernel(x_hbm, k_hbm, v_hbm, wq_hbm, wo_hbm, wg_hbm, wu_hbm, wd_hbm, c_hbm, wm_hbm, o_hbm,
            x_v, k_v, v_v, wq_v, wo_v, wg_v, wu_v, wd_v, c_v, wm_v, out_v,
            mod_v, sc_v, h_v, acc_v, s0_v, s1_v, m_c, o_c, l_c, h2_v,
            sem_head, sem_misc, sem_x, sem_out):
    scale = (DH ** -0.5) * LOG2E
    s_refs = (s0_v, s1_v)

    def head_copies(h, slot):
        col = pl.multiple_of(h * DH, DH)
        return [
            pltpu.make_async_copy(wq_hbm.at[:, pl.ds(col, DH)], wq_v.at[slot], sem_head.at[0, slot]),
            pltpu.make_async_copy(k_hbm.at[h], k_v.at[slot], sem_head.at[1, slot]),
            pltpu.make_async_copy(v_hbm.at[h], v_v.at[slot], sem_head.at[2, slot]),
            pltpu.make_async_copy(wo_hbm.at[h], wo_v.at[slot], sem_head.at[3, slot]),
        ]

    cp_c = pltpu.make_async_copy(c_hbm, c_v, sem_misc.at[0])
    cp_wm0 = pltpu.make_async_copy(wm_hbm.at[:, pl.ds(0, 2 * D)], wm_v.at[:, pl.ds(0, 2 * D)], sem_misc.at[1])
    cp_wm1 = pltpu.make_async_copy(wm_hbm.at[:, pl.ds(2 * D, 4 * D)], wm_v.at[:, pl.ds(2 * D, 4 * D)],
                                   sem_misc.at[2])
    cp_ffn = [cp_wm1,
              pltpu.make_async_copy(wg_hbm, wg_v, sem_misc.at[3]),
              pltpu.make_async_copy(wu_hbm, wu_v, sem_misc.at[4]),
              pltpu.make_async_copy(wd_hbm, wd_v, sem_misc.at[5])]
    cp_x = [pltpu.make_async_copy(x_hbm.at[pl.ds(i * XR, XR), :], x_v.at[pl.ds(i * XR, XR), :], sem_x.at[i])
            for i in range(XC)]

    def out_copy(i):
        rows = pl.ds(pl.multiple_of(i * RF, RF), RF)
        return pltpu.make_async_copy(out_v.at[rows, :], o_hbm.at[rows, :], sem_out.at[i])

    def ln1(c):
        sa = mod_v[0:1, 0:D]
        ca1 = 1.0 + mod_v[0:1, D:2 * D]
        rows = pl.ds(c * R, R)
        h_v[rows, :] = (_layernorm(x_v[rows, :].astype(f32)) * ca1 + sa).astype(bf16)

    def ffn_mods():
        ga = mod_v[0:1, 2 * D:3 * D]
        sb = mod_v[0:1, 3 * D:4 * D]
        cb1 = 1.0 + mod_v[0:1, 4 * D:5 * D]
        gb = mod_v[0:1, 5 * D:6 * D]
        return ga, sb, cb1, gb

    def ln2(i, r0, nr, dst):
        ga, sb, cb1, _ = ffn_mods()
        rows = pl.ds(pl.multiple_of(i * RF + r0, 16), nr)
        x2 = x_v[rows, :].astype(f32) + ga * acc_v[rows, :]
        dst[pl.ds(r0, nr), :] = (_layernorm(x2) * cb1 + sb).astype(bf16)

    class Heads:
        def __init__(self, h0, c0):
            self.h0, self.c0, self.cache = h0, c0, {}

        def views(self, t):
            dh = (self.c0 + t) // N
            if dh not in self.cache:
                slot = (self.h0 + dh) & (NSLOT - 1)
                self.cache[dh] = dict(k=k_v.at[slot], v=v_v.at[slot], wq=wq_v.at[slot], wo=wo_v.at[slot])
            return self.cache[dh]

        def rows(self, t):
            return pl.ds(((self.c0 + t) % N) * R, R)

    def qproj(hd, t):
        q = jnp.dot(h_v[hd.rows(t), :], hd.views(t)['wq'][...], preferred_element_type=f32)
        return (q * scale).astype(bf16)

    def scores(q, hd, t, k0, nk, sref, z):
        s = lax.dot_general(q, hd.views(t)['k'][pl.ds(k0, nk), :], (((1,), (1,)), ((), ())),
                            preferred_element_type=f32)
        sref[z, :, pl.ds(k0, nk)] = s
        lt = _lane_tiles(s)
        mm = lt[0]
        for x in lt[1:]:
            mm = jnp.maximum(mm, x)
        return mm

    def rowmax(mp):
        return jnp.max(mp, axis=-1, keepdims=True)

    def normalize(o, lp):
        l = jnp.sum(lp, axis=-1, keepdims=True)
        return (o * _reciprocal(l)).astype(bf16)

    def oproj(on, hd, t):
        acc_v[hd.rows(t), :] += jnp.dot(on, hd.views(t)['wo'][...], preferred_element_type=f32)

    def run_positions(hd, n, st, z0, z1, sched, last=False, hook=None):
        def exists(t):
            return not last or t < n

        from_scratch = st is None
        m = {} if from_scratch else {0: st[0]}
        o_prev = l_prev = o = lp = on = q = None
        assert sched['q'] < sched['a']
        for t in range(n):
            has_prev = t > 0 or from_scratch or st[1] is not None
            for j in range(G):
                if hook is not None:
                    hook(t, j)
                if sched['q'] < 0 and j == 0 and exists(t + 1):
                    q = qproj(hd, t + 1)
                if j == sched['a'] and exists(t + 1):
                    m[t + 1] = rowmax(scores(q, hd, t + 1, 0, S, s_refs[(hd.c0 + t + 1) % 2], z0))
                sv = s_refs[(hd.c0 + t) % 2][z1, :, pl.ds(j * W, W)]
                if t == 0 and from_scratch:
                    if j == 0:
                        m[0] = m_c[...]
                    e = jnp.concatenate([jnp.exp2(x - m[0]) for x in _lane_tiles(sv)], axis=1)
                else:
                    e = jnp.exp2(sv - m[t])
                for i, x in enumerate(_lane_tiles(e)):
                    lp = x if (j == 0 and i == 0) else lp + x
                pv = jnp.dot(e.astype(bf16), hd.views(t)['v'][pl.ds(j * W, W), :], preferred_element_type=f32)
                o = pv if j == 0 else o + pv
                if j == sched['n'] and has_prev:
                    if t == 0:
                        o_prev, l_prev = (o_c[...], l_c[...]) if from_scratch else (st[1], st[2])
                    on = normalize(o_prev, l_prev)
                if j == sched['o'] and has_prev:
                    oproj(on, hd, t - 1)
                if j == sched['q'] and exists(t + 1):
                    q = qproj(hd, t + 1)
            o_prev, l_prev = o, lp
        if last:
            oproj(normalize(o_prev, l_prev), hd, n - 1)
            return None
        return m[n], o_prev, l_prev

    def save_state(st):
        m_c[...] = jnp.broadcast_to(st[0], (R, 128))
        o_c[...] = st[1]
        l_c[...] = st[2]

    cp_wq0, cp_k0, cp_v0, cp_wo0 = head_copies(0, 0)
    for cp in (cp_c, cp_wm0, cp_x[0], cp_x[1], cp_wq0, cp_k0):
        cp.start()

    za = lax.fori_loop(0, 2, lambda i, c: c + lax.shift_right_logical(i, 6), 0)
    zb = lax.shift_right_logical(za, 1)

    acc_v[...] = jnp.zeros_like(acc_v)
    cp_c.wait()
    cval = c_v[...].astype(f32)
    sc_v[...] = jnp.broadcast_to((cval * jax.nn.sigmoid(cval)).astype(bf16), (16, D))
    cp_wm0.wait()
    for cp in (cp_x[2], cp_x[3], cp_v0):
        cp.start()
    cp_x[0].wait()
    cp_x[1].wait()
    cp_wq0.wait()
    cp_wo0.start()
    mod_v[:, pl.ds(0, 2 * D)] = jnp.dot(sc_v[...], wm_v[:, pl.ds(0, 2 * D)], preferred_element_type=f32)
    ln1(0)
    head0 = Heads(0, 0)
    q0 = qproj(head0, 0)
    cp_k0.wait()
    for cp in cp_x[4:]:
        cp.start()

    mp0 = None
    for j in range(G):
        mm0 = scores(q0, head0, 0, j * W, W, s0_v, za)
        mp0 = mm0 if j == 0 else jnp.maximum(mp0, mm0)
        if j == 1:
            cp_x[2].wait()
            cp_x[3].wait()
            ln1(1)
    m0 = rowmax(mp0)

    def first_hook(t, j):
        if j == 0 and t + 2 < N:
            if t == 0:
                cp_v0.wait()
                cp_wo0.wait()
            cp_x[4 + 2 * t].wait()
            cp_x[5 + 2 * t].wait()
            if t == 0:
                for cp in head_copies(1, 1) + head_copies(2, 2):
                    cp.start()
            ln1(t + 2)

    save_state(run_positions(head0, RHO, (m0, None, None), za, zb, SCHED_EDGE, hook=first_hook))

    def head_body(h, carry):
        for cp in head_copies(h + 1, (h + 1) & (NSLOT - 1)):
            cp.wait()

        @pl.when(h == 0)
        def _():
            for cp in cp_ffn:
                cp.start()

        z0 = lax.shift_right_logical(h, 6)
        z1 = lax.shift_right_logical(h, 7)
        save_state(run_positions(Heads(h, RHO), N, None, z0, z1, SCHED_LOOP))
        h3 = h + 3

        @pl.when(h3 < H)
        def _():
            for cp in head_copies(jnp.minimum(h3, H - 1), h3 & (NSLOT - 1)):
                cp.start()

        return carry

    lax.fori_loop(0, H - 1, head_body, 0)

    for cp in cp_ffn:
        cp.wait()
    mod_v[:, pl.ds(2 * D, 4 * D)] = jnp.dot(sc_v[...], wm_v[:, pl.ds(2 * D, 4 * D)], preferred_element_type=f32)

    def last_hook(t, j):
        if t == 0 and j == 0:
            ln2(0, 0, RF, h2_v.at[0])

    run_positions(Heads(H - 1, RHO), N - RHO, None, za, zb, SCHED_EDGE, last=True, hook=last_hook)

    def ffn_body(i, carry):
        ga, _, _, gb = ffn_mods()
        src = h2_v.at[i & 1]
        dst = h2_v.at[(i + 1) & 1]
        nxt = jnp.minimum(i + 1, NF - 1)
        y = None
        for j in range(F // FW):
            cols = pl.ds(j * FW, FW)
            h2 = src[...]
            g = jnp.dot(h2, wg_v[:, cols], preferred_element_type=f32)
            u = jnp.dot(h2, wu_v[:, cols], preferred_element_type=f32)
            a = (jax.nn.gelu(g, approximate=True) * u).astype(bf16)
            t = jnp.dot(a, wd_v[cols, :], preferred_element_type=f32)
            y = t if j == 0 else y + t
            if j in (2, 3):
                ln2(nxt, (j - 2) * (RF // 2), RF // 2, dst)
        rows = pl.ds(pl.multiple_of(i * RF, RF), RF)
        x2 = x_v[rows, :].astype(f32) + ga * acc_v[rows, :]
        out_v[rows, :] = (x2 + gb * y).astype(bf16)
        out_copy(i).start()
        return carry

    lax.fori_loop(0, NF, ffn_body, 0)
    for i in range(NF):
        out_copy(i).wait()


@jax.jit
def pallas_adaLN_cond__mha_block_cached__geglu_ffn__prompt_kernel(
    A_x: jax.Array,
    A_k_cache: jax.Array,
    A_v_cache: jax.Array,
    A_wq: jax.Array,
    A_wo: jax.Array,
    B_x: jax.Array,
    B_w_gate: jax.Array,
    B_w_up: jax.Array,
    B_w_down: jax.Array,
    c: jax.Array,
    w_mod: jax.Array,
):
    del B_x
    hbm = pl.BlockSpec(memory_space=pl.ANY)
    out = pl.pallas_call(
        _kernel,
        in_specs=[hbm] * 10,
        out_specs=hbm,
        out_shape=jax.ShapeDtypeStruct((S, D), bf16),
        scratch_shapes=[
            pltpu.VMEM((S, D), bf16),
            pltpu.VMEM((NSLOT, S, DH), bf16),
            pltpu.VMEM((NSLOT, S, DH), bf16),
            pltpu.VMEM((NSLOT, D, DH), bf16),
            pltpu.VMEM((NSLOT, DH, D), bf16),
            pltpu.VMEM((D, F), bf16),
            pltpu.VMEM((D, F), bf16),
            pltpu.VMEM((F, D), bf16),
            pltpu.VMEM((1, D), bf16),
            pltpu.VMEM((D, 6 * D), bf16),
            pltpu.VMEM((S, D), bf16),
            pltpu.VMEM((16, 6 * D), f32),
            pltpu.VMEM((16, D), bf16),
            pltpu.VMEM((S, D), bf16),
            pltpu.VMEM((S, D), f32),
            pltpu.VMEM((2, R, S), f32),
            pltpu.VMEM((2, R, S), f32),
            pltpu.VMEM((R, 128), f32),
            pltpu.VMEM((R, DH), f32),
            pltpu.VMEM((R, 128), f32),
            pltpu.VMEM((2, RF, D), bf16),
            pltpu.SemaphoreType.DMA((4, NSLOT)),
            pltpu.SemaphoreType.DMA((6,)),
            pltpu.SemaphoreType.DMA((XC,)),
            pltpu.SemaphoreType.DMA((NF,)),
        ],
        compiler_params=pltpu.CompilerParams(
            vmem_limit_bytes=100 * 1024 * 1024,
            disable_bounds_checks=True,
            disable_semaphore_checks=True,
            flags={"XLA_TPU_FORCE_LP_LLO_SCHEDULER": True},
        ),
    )(
        A_x.reshape(S, D),
        A_k_cache.reshape(H, S, DH),
        A_v_cache.reshape(H, S, DH),
        A_wq,
        A_wo.reshape(H, DH, D),
        B_w_gate,
        B_w_up,
        B_w_down,
        c,
        w_mod,
    )
    return out.reshape(1, S, D)
```
